```python
import jax
import jax.numpy as jnp

def _softmax(x, axis=-1):
    return jax.nn.softmax(x, axis=axis)
def _gelu(x):
    return jax.nn.gelu(x, approximate=True)
def _silu(x):
    return jax.nn.silu(x)
def _sigmoid(x):
    return jax.nn.sigmoid(x)
def _layernorm(x, axis=-1, eps=1e-5):
    m = jnp.mean(x, axis=axis, keepdims=True)
    v = jnp.var(x, axis=axis, keepdims=True)
    return (x - m) / jnp.sqrt(v + eps)
def _scatter_add(tgt, idx, src, axis=0):
    return tgt.at[idx].add(src)
def _segment_sum(src, seg, n):
    return jax.ops.segment_sum(src, seg, n)
class _Rng:
    def __init__(self, key):
        self._k = key
    def _next(self):
        self._k, sub = jax.random.split(self._k)
        return sub
    def normal(self, shape):
        return jax.random.normal(self._next(), shape, dtype=jnp.bfloat16)
    def randint(self, lo, hi, shape):
        return jax.random.randint(self._next(), shape, lo, hi, dtype=jnp.int32)
    def uniform(self, shape, lo=0.0, hi=1.0):
        return jax.random.uniform(self._next(), shape, jnp.bfloat16, lo, hi)
    def permutation(self, n):
        return jax.random.permutation(self._next(), n)


kernel_name = 'concat_heads__compressed_kv_cla__mha_block_cached__decode'

def setup_inputs():
    _rng = _Rng(jax.random.key(int.from_bytes(__import__("os").urandom(4), "little")))
    _w = (lambda a: (lambda t: t.astype(jnp.bfloat16) if jnp.issubdtype(t.dtype, jnp.floating) else t)(jnp.asarray(a)))
    def _A_setup():
        B, H, Sq, Sk, D, M = 4, 32, 1, 4096, 128, 512
        Dc = 4 * D
        return {
            "x": _w((lambda *s: _rng.normal(s) * 0.05)(B, Sq, M)),
            "c_kv": _w((lambda *s: _rng.normal(s) * 0.05)(B, Sk, Dc)),
            "w_q": _w((lambda *s: _rng.normal(s) * 0.05)(M, H, D) * (M ** -0.5)),
            "w_uk": _w((lambda *s: _rng.normal(s) * 0.05)(Dc, H, D) * (Dc ** -0.5)),
            "w_uv": _w((lambda *s: _rng.normal(s) * 0.05)(Dc, H, D) * (Dc ** -0.5)),
            "w_o": _w((lambda *s: _rng.normal(s) * 0.05)(H, D, M) * ((H * D) ** -0.5)),
        }
    _A_in = _A_setup()

    def _B_setup():
        B, Sq, D = 4, 1, 512
        H, Sk, Dh = 32, 4096, 128
        return {
            "x": _w((lambda *s: _rng.normal(s) * 0.05)(B, Sq, D)),
            "k_cache": _w((lambda *s: _rng.normal(s) * 0.05)(B, H, Sk, Dh)),
            "v_cache": _w((lambda *s: _rng.normal(s) * 0.05)(B, H, Sk, Dh)),
            "wq": _w((lambda *s: _rng.normal(s) * 0.05)(D, H * Dh) * (D ** -0.5)),
            "wo": _w((lambda *s: _rng.normal(s) * 0.05)(H * Dh, D) * ((H * Dh) ** -0.5)),
        }
    _B_in = _B_setup()

    return {
        "A_x": _A_in["x"],
        "A_c_kv": _A_in["c_kv"],
        "A_w_q": _A_in["w_q"],
        "A_w_uk": _A_in["w_uk"],
        "A_w_uv": _A_in["w_uv"],
        "A_w_o": _A_in["w_o"],
        "B_x": _B_in["x"],
        "B_k_cache": _B_in["k_cache"],
        "B_v_cache": _B_in["v_cache"],
        "B_wq": _B_in["wq"],
        "B_wo": _B_in["wo"],
    }

def reference(A_x, A_c_kv, A_w_q, A_w_uk, A_w_uv, A_w_o, B_x, B_k_cache, B_v_cache, B_wq, B_wo):
    def _A_ref(x, c_kv, w_q, w_uk, w_uv, w_o):
        B, Sq, M = x.shape[0], x.shape[1], x.shape[2]
        Sk = c_kv.shape[1]
        H, D = w_q.shape[1], w_q.shape[2]
        q = jnp.einsum("bqm,mhd->bhqd", x, w_q)
        k = jnp.einsum("bkc,chd->bhkd", c_kv, w_uk)
        v = jnp.einsum("bkc,chd->bhkd", c_kv, w_uv)
        scores = jnp.einsum("bhqd,bhkd->bhqk", q, k) * (D ** -0.5)
        off = Sk - Sq
        qi = jnp.arange(Sq)[:, None]
        kj = jnp.arange(Sk)[None, :]
        cmask = kj <= (qi + off)
        scores = jnp.where(cmask[None, None], scores, -1e9)
        p = _softmax(scores, axis=-1)
        ctx = jnp.einsum("bhqk,bhkd->bhqd", p, v)
        return jnp.einsum("bhqd,hdm->bqm", ctx, w_o)

    def _B_ref(x, k_cache, v_cache, wq, wo):
        B, Sq, D = x.shape
        H, Dh = 32, 128
        q = (lambda x, *d: x.transpose(*d))((x @ wq).reshape(B, Sq, H, Dh), 0, 2, 1, 3)
        scores = jnp.einsum("bhqd,bhkd->bhqk", q, k_cache) * (Dh ** -0.5)
        p = _softmax(scores, axis=-1)
        o = jnp.einsum("bhqk,bhkd->bhqd", p, v_cache)
        return (lambda x, *d: x.transpose(*d))(o, 0, 2, 1, 3).reshape(B, Sq, H * Dh) @ wo

    a = _A_ref(A_x, A_c_kv, A_w_q, A_w_uk, A_w_uv, A_w_o)
    b = _B_ref(B_x, B_k_cache, B_v_cache, B_wq, B_wo)
    return jnp.concatenate([a, b], axis=-1)
```

```python
import functools

import jax
import jax.numpy as jnp
from jax import lax
import jax.experimental.pallas as pl
import jax.experimental.pallas.tpu as pltpu

F32 = jnp.float32
BF16 = jnp.bfloat16

B = 4
H = 32
SK = 4096
D = 128
M = 512
HG = 8
NG = B * H // HG
R = 512
NC = SK // R
ND = 32
SUB = R // ND
LOOK = 2
NSLOT = LOOK + 1
SCALE = float(D) ** -0.5

NT = (((1,), (1,)), ((), ()))


def _kernel(
    xa_hbm, ckv_hbm, wqa_hbm, wuk_hbm, wuv_hbm, woa_hbm,
    xb_hbm, k_hbm, v_hbm, wqb_hbm, wob_hbm,
    out_ref,
    kbuf, vbuf, ckv, wqa, wuk, wuv, woa, wqb, wob, xa, xb,
    e_ref, qb_s, s_buf, p_buf, linv, acc, ob,
    ya, pacc, qa, qabs, sa, pa, linva, acca, oa, outa, outb,
    ksem, vsem, wsem, osem, xsem,
):
    def k_desc(g, c, d, slot):
        return pltpu.make_async_copy(
            k_hbm.at[g // 4, pl.ds((g % 4) * HG, HG), pl.ds(c * R + d * SUB, SUB)],
            kbuf.at[slot, :, pl.ds(d * SUB, SUB)], ksem.at[slot])

    def v_desc(g, c, d, slot):
        return pltpu.make_async_copy(
            v_hbm.at[g // 4, pl.ds((g % 4) * HG, HG), pl.ds(c * R + d * SUB, SUB)],
            vbuf.at[slot, :, pl.ds(d * SUB, SUB)], vsem.at[slot])

    def ckv_desc(s, d):
        r = pl.multiple_of((s * ND + d) * 8, 8)
        return pltpu.make_async_copy(
            ckv_hbm.at[:, pl.ds(r, 8)], ckv.at[:, pl.ds(r, 8)], wsem.at[0])

    def w3_desc(src, dst, sem):
        def f(s, d):
            r = pl.multiple_of((s * ND + d) * 32, 32)
            return pltpu.make_async_copy(
                src.at[:, pl.ds(r, 32)], dst.at[:, pl.ds(r, 32)], sem)
        return f

    wqa_desc = w3_desc(wqa_hbm, wqa, wsem.at[1])
    wuk_desc = w3_desc(wuk_hbm, wuk, wsem.at[2])
    wuv_desc = w3_desc(wuv_hbm, wuv, wsem.at[3])

    def wqb_desc(s, d):
        r = pl.multiple_of((s * 4 + d // 8) * 8, 8)
        col = (d % 8) * 512
        return pltpu.make_async_copy(
            wqb_hbm.at[:, pl.ds(r, 8), pl.ds(col, 512)],
            wqb.at[:, pl.ds(r, 8), pl.ds(col, 512)], wsem.at[4])

    def wo_desc(src, dst, base):
        def f(s, d):
            r = pl.multiple_of((s * ND + d) * 8, 8)
            return pltpu.make_async_copy(
                src.at[:, pl.ds(r, 8)], dst.at[:, pl.ds(r, 8)], osem.at[base + s])
        return f

    wob_desc = wo_desc(wob_hbm, wob, 0)
    woa_desc = wo_desc(woa_hbm, woa, 4)

    def issue(lane0, lane1):
        for d in range(ND):
            lane0(d).start(priority=0)
            lane1(d).start(priority=1)

    def wait_all(ref, sem):
        pltpu.make_async_copy(ref, ref, sem).wait()

    def issue_pro(desc0, n0, lo=0, hi=4):
        def body(s, carry):
            issue(functools.partial(desc0, s), functools.partial(ckv_desc, n0 + s))
            return carry
        lax.fori_loop(lo, hi, body, 0)

    def issue_step(u):
        gu = u // NC
        cu = u % NC
        slot = u % NSLOT
        kd = lambda d: k_desc(gu, cu, d, slot)
        vd = lambda d: v_desc(gu - 1, cu, d, slot)

        @pl.when(jnp.logical_and(u >= NC, u < NG * NC))
        def _():
            issue(kd, vd)

        @pl.when(u < 4)
        def _():
            issue(kd, functools.partial(ckv_desc, 12 + u))

        @pl.when(jnp.logical_and(u >= 4, u < NC))
        def _():
            issue(kd, functools.partial(wuv_desc, u - 4))

        @pl.when(jnp.logical_and(u >= NG * NC, u < NG * NC + 4))
        def _():
            issue(functools.partial(wob_desc, u - NG * NC), vd)

        @pl.when(jnp.logical_and(u >= NG * NC + 4, u < (NG + 1) * NC))
        def _():
            issue(functools.partial(woa_desc, u - NG * NC - 4), vd)

    issue_pro(wqb_desc, 0, 0, 1)
    xa_cp = pltpu.make_async_copy(xa_hbm, xa, xsem.at[0])
    xb_cp = pltpu.make_async_copy(xb_hbm, xb, xsem.at[1])
    xa_cp.start()
    xb_cp.start()

    er = lax.broadcasted_iota(jnp.int32, (128, 1024), 0)
    ec = lax.broadcasted_iota(jnp.int32, (128, 1024), 1)
    for j in range(4):
        e_ref[:, j * 1024:(j + 1) * 1024] = jnp.where(
            (ec // H) + j * 32 == er, 1.0, 0.0).astype(BF16)
    ob[...] = jnp.zeros_like(ob)
    oa[...] = jnp.zeros_like(oa)
    outa[...] = jnp.zeros_like(outa)
    outb[...] = jnp.zeros_like(outb)

    issue_pro(wqb_desc, 0, 1, 4)
    issue_pro(wqa_desc, 4, 0, 2)

    xa_cp.wait()
    xb_cp.wait()
    row8 = lax.broadcasted_iota(jnp.int32, (8, M), 0)
    xb8 = jnp.zeros((8, M), F32)
    for b in range(B):
        xb8 = jnp.where(row8 == b, xb[b].astype(F32), xb8)
        ya[b * H:(b + 1) * H, :] = jnp.broadcast_to(
            xa[b].astype(F32), (H, M)).astype(BF16)
    xb8 = xb8.astype(BF16)

    wait_all(wqb, wsem.at[4])
    qb = jnp.dot(xb8[:, 0:128], wqb[0], preferred_element_type=F32)
    for kc in range(1, 4):
        qb += jnp.dot(xb8[:, kc * 128:(kc + 1) * 128], wqb[kc],
                      preferred_element_type=F32)
    for h in range(H):
        qb_s[pl.ds(h, B, stride=H), :] = qb[0:B, h * D:(h + 1) * D]

    issue_pro(wqa_desc, 4, 2, 4)
    issue_pro(wuk_desc, 8, 0, 4)
    for u in range(LOOK):
        issue(lambda d: k_desc(0, u, d, u % NSLOT),
              functools.partial(ckv_desc, 12 + u))

    def hmask():
        r = lax.broadcasted_iota(jnp.int32, (128, 1024), 0)
        c = lax.broadcasted_iota(jnp.int32, (128, 1024), 1)
        return (r % H) == (c % H)

    def proj_piece(w_ref, kc):
        y = ya[:, pl.ds(pl.multiple_of(kc * 128, 128), 128)]
        msk = hmask()
        tot = None
        for j in range(4):
            lx = jnp.dot(y, e_ref[:, j * 1024:(j + 1) * 1024],
                         preferred_element_type=F32)
            lx = jnp.where(msk, lx, 0.0).astype(BF16)
            t = jnp.dot(lx, w_ref[kc, j * 1024:(j + 1) * 1024, :],
                        preferred_element_type=F32)
            tot = t if tot is None else tot + t

        @pl.when(kc == 0)
        def _():
            pacc[...] = tot

        @pl.when(kc > 0)
        def _():
            pacc[...] += tot

    def qabs_piece(kc):
        q = qa[...]
        msk = hmask()
        tot = None
        for j in range(4):
            gx = lax.dot_general(q, wuk[kc, j * 1024:(j + 1) * 1024, :], NT,
                                 preferred_element_type=F32)
            gx = jnp.where(msk, gx, 0.0).astype(BF16)
            t = lax.dot_general(gx, e_ref[:, j * 1024:(j + 1) * 1024], NT,
                                preferred_element_type=F32)
            tot = t if tot is None else tot + t
        qabs[:, pl.ds(pl.multiple_of(kc * 128, 128), 128)] = tot.astype(BF16)

    def a_scores(b, c):
        off = pl.multiple_of(c * 1024, 1024)
        q = qabs[pl.ds(pl.multiple_of(b * H, H), H), :]
        sa[:, pl.ds(off, 1024)] = lax.dot_general(
            q, ckv[b, pl.ds(off, 1024), :], NT, preferred_element_type=F32)

    def a_softmax():
        s = sa[...]
        m = jnp.max(s, axis=1, keepdims=True)
        p = jnp.exp((s - m) * SCALE)
        pa[...] = p.astype(BF16)
        linva[...] = jnp.broadcast_to(
            1.0 / jnp.sum(p, axis=1, keepdims=True), linva.shape)

    def a_pv(b, c):
        off = pl.multiple_of(c * 1024, 1024)
        t = jnp.dot(pa[:, pl.ds(off, 1024)], ckv[b, pl.ds(off, 1024), :],
                    preferred_element_type=F32)

        @pl.when(c == 0)
        def _():
            acca[...] = t

        @pl.when(c > 0)
        def _():
            acca[...] += t

    def out_piece(o_ref, w_ref, s, regions):
        tot = None
        for r in regions:
            for jj in range(2):
                lhs = o_ref[r * HG + 2 * s + jj].astype(BF16)
                off = pl.multiple_of((2 * s + jj) * D, D)
                t = jnp.dot(lhs, w_ref[r, pl.ds(off, D), :],
                            preferred_element_type=F32)
                tot = t if tot is None else tot + t
        return tot

    def step(t, carry):
        g = t // NC
        c = t % NC
        slot = t % NSLOT
        off = pl.multiple_of(c * R, R)

        issue_step(t + LOOK)

        @pl.when(g >= 1)
        def _pv():
            wait_all(vbuf.at[slot], vsem.at[slot])
            p = p_buf[:, pl.ds(off, R)].astype(BF16)
            for j in range(HG):
                acc[j] += jnp.dot(p, vbuf[slot, j], preferred_element_type=F32)

            @pl.when(c == NC - 1)
            def _():
                gp = g - 1
                for j in range(HG):
                    o = acc[j] * linv[...]
                    ob[(gp % 4) * HG + j, pl.ds(gp // 4, 1), :] = o[j:j + 1, :]

        @pl.when(g < NG)
        def _qk():
            wait_all(kbuf.at[slot], ksem.at[slot])
            q = qb_s[pl.ds(pl.multiple_of(g * HG, HG), HG), :].astype(BF16)
            row = lax.broadcasted_iota(jnp.int32, (HG, R), 0)
            s = None
            for j in range(HG):
                r = lax.dot_general(q, kbuf[slot, j], NT,
                                    preferred_element_type=F32)
                s = r if s is None else jnp.where(row == j, r, s)
            s_buf[:, pl.ds(off, R)] = s

            @pl.when(c == NC - 1)
            def _():
                sv = s_buf[...]
                m = jnp.max(sv, axis=1, keepdims=True)
                p = jnp.exp((sv - m) * SCALE)
                p_buf[...] = p
                linv[...] = jnp.broadcast_to(
                    1.0 / jnp.sum(p, axis=1, keepdims=True), linv.shape)
                acc[...] = jnp.zeros_like(acc)

        @pl.when(t == NC)
        def _():
            wait_all(wqa, wsem.at[1])
            wait_all(wuk, wsem.at[2])
            wait_all(wuv, wsem.at[3])
            wait_all(ckv, wsem.at[0])

        @pl.when(jnp.logical_and(g == 1, c < 4))
        def _():
            proj_piece(wqa, c)

            @pl.when(c == 3)
            def _():
                qa[...] = pacc[...].astype(BF16)

        @pl.when(jnp.logical_and(g == 1, c >= 4))
        def _():
            qabs_piece(c - 4)

        a_attn = jnp.logical_and(g >= 2, g < 2 + B)

        @pl.when(jnp.logical_and(a_attn, c < 4))
        def _():
            a_scores(g - 2, c)

            @pl.when(c == 3)
            def _():
                a_softmax()

        @pl.when(jnp.logical_and(a_attn, c >= 4))
        def _():
            a_pv(g - 2, c - 4)

            @pl.when(c == NC - 1)
            def _():
                li = linva[...]
                li = jnp.concatenate([li] * 4, axis=1)
                ya[pl.ds(pl.multiple_of((g - 2) * H, H), H), :] = (
                    acca[...] * li).astype(BF16)

        @pl.when(jnp.logical_and(g == 2 + B, c < 4))
        def _():
            proj_piece(wuv, c)

            @pl.when(c == 3)
            def _():
                for h in range(H):
                    oa[h, 0:B, :] = pacc[pl.ds(h, B, stride=H), :]

        @pl.when(jnp.logical_and(g == NG, c < 4))
        def _():
            rows = pl.ds(pl.multiple_of(c * 256, 256), 256)
            wait_all(wob.at[:, rows], osem.at[c])
            outb[...] += out_piece(ob, wob, c, (0, 1, 2))

        @pl.when(jnp.logical_and(g == NG, c >= 4))
        def _():
            rows = pl.ds(pl.multiple_of((c - 4) * 256, 256), 256)
            wait_all(woa.at[:, rows], osem.at[c])
            outa[...] += out_piece(oa, woa, c - 4, (0, 1, 2, 3))

        return carry

    lax.fori_loop(0, (NG + 1) * NC, step, 0)

    resb = outb[...]
    for s in range(4):
        resb += out_piece(ob, wob, s, (3,))
    resa = outa[...]
    for b in range(B):
        out_ref[b, :, 0:M] = resa[b:b + 1, :].astype(out_ref.dtype)
        out_ref[b, :, M:2 * M] = resb[b:b + 1, :].astype(out_ref.dtype)


@jax.jit
def pallas_concat_heads__compressed_kv_cla__mha_block_cached__decode_kernel(
    A_x: jax.Array,
    A_c_kv: jax.Array,
    A_w_q: jax.Array,
    A_w_uk: jax.Array,
    A_w_uv: jax.Array,
    A_w_o: jax.Array,
    B_x: jax.Array,
    B_k_cache: jax.Array,
    B_v_cache: jax.Array,
    B_wq: jax.Array,
    B_wo: jax.Array,
):
    wqa = A_w_q.reshape(4, 128 * H, D)
    wuk = A_w_uk.reshape(4, 128 * H, D)
    wuv = A_w_uv.reshape(4, 128 * H, D)
    woa = A_w_o.reshape(4, HG * D, M)
    wqb = B_wq.reshape(4, 128, H * D)
    wob = B_wo.reshape(4, HG * D, M)

    vm = pltpu.VMEM
    scratch = [
        vm((NSLOT, HG, R, D), BF16),
        vm((NSLOT, HG, R, D), BF16),
        vm((B, SK, M), BF16),
        vm((4, 128 * H, D), BF16),
        vm((4, 128 * H, D), BF16),
        vm((4, 128 * H, D), BF16),
        vm((4, HG * D, M), BF16),
        vm((4, 128, H * D), BF16),
        vm((4, HG * D, M), BF16),
        vm((B, 1, M), BF16),
        vm((B, 1, M), BF16),
        vm((128, 128 * H), BF16),
        vm((B * H, D), F32),
        vm((HG, SK), F32),
        vm((HG, SK), F32),
        vm((HG, D), F32),
        vm((HG, HG, D), F32),
        vm((H, 8, D), F32),
        vm((B * H, M), BF16),
        vm((B * H, D), F32),
        vm((B * H, D), BF16),
        vm((B * H, M), BF16),
        vm((H, SK), F32),
        vm((H, SK), BF16),
        vm((H, D), F32),
        vm((H, M), F32),
        vm((H, 8, D), F32),
        vm((8, M), F32),
        vm((8, M), F32),
        pltpu.SemaphoreType.DMA((NSLOT,)),
        pltpu.SemaphoreType.DMA((NSLOT,)),
        pltpu.SemaphoreType.DMA((5,)),
        pltpu.SemaphoreType.DMA((8,)),
        pltpu.SemaphoreType.DMA((2,)),
    ]
    return pl.pallas_call(
        _kernel,
        in_specs=[pl.BlockSpec(memory_space=pl.ANY)] * 11,
        out_specs=pl.BlockSpec(memory_space=pltpu.VMEM),
        out_shape=jax.ShapeDtypeStruct((B, 1, 2 * M), A_x.dtype),
        scratch_shapes=scratch,
        compiler_params=pltpu.CompilerParams(
            vmem_limit_bytes=96 * 1024 * 1024),
    )(A_x, A_c_kv, wqa, wuk, wuv, woa, B_x, B_k_cache, B_v_cache, wqb, wob)
```

```python
import functools

import jax
import jax.numpy as jnp
from jax import lax
import jax.experimental.pallas as pl
import jax.experimental.pallas.tpu as pltpu

F32 = jnp.float32
BF16 = jnp.bfloat16

B = 4
H = 32
SK = 4096
D = 128
M = 512
HG = 8
NG = B * H // HG
R = 512
NC = SK // R
ND = 32
SUB = R // ND
LOOK = 2
NSLOT = LOOK + 1
SCALE = float(D) ** -0.5

NT = (((1,), (1,)), ((), ()))


def _kernel(
    xa_hbm, ckv_hbm, wqa_hbm, wuk_hbm, wuv_hbm, woa_hbm,
    xb_hbm, k_hbm, v_hbm, wqb_hbm, wob_hbm,
    out_ref,
    kbuf, vbuf, ckv, wqa, wuk, wuv, woa, wqb, wob, xa, xb,
    e_ref, qb_s, s_buf, p_buf, linv, acc, ob,
    ya, pacc, qa, qabs, sa, pa, linva, acca, oa, outa, outb,
    ksem, vsem, wsem, osem, xsem,
):
    def k_desc(g, c, d, slot):
        return pltpu.make_async_copy(
            k_hbm.at[g // 4, pl.ds((g % 4) * HG, HG), pl.ds(c * R + d * SUB, SUB)],
            kbuf.at[slot, :, pl.ds(d * SUB, SUB)], ksem.at[slot])

    def v_desc(g, c, d, slot):
        return pltpu.make_async_copy(
            v_hbm.at[g // 4, pl.ds((g % 4) * HG, HG), pl.ds(c * R + d * SUB, SUB)],
            vbuf.at[slot, :, pl.ds(d * SUB, SUB)], vsem.at[slot])

    def ckv_desc(s, d):
        r = pl.multiple_of((s * ND + d) * 8, 8)
        return pltpu.make_async_copy(
            ckv_hbm.at[:, pl.ds(r, 8)], ckv.at[:, pl.ds(r, 8)], wsem.at[0])

    def w3_desc(src, dst, sem):
        def f(s, d):
            r = pl.multiple_of((s * ND + d) * 32, 32)
            return pltpu.make_async_copy(
                src.at[:, pl.ds(r, 32)], dst.at[:, pl.ds(r, 32)], sem)
        return f

    wqa_desc = w3_desc(wqa_hbm, wqa, wsem.at[1])
    wuk_desc = w3_desc(wuk_hbm, wuk, wsem.at[2])
    wuv_desc = w3_desc(wuv_hbm, wuv, wsem.at[3])

    def wqb_desc(s, d):
        r = pl.multiple_of((s * 4 + d // 8) * 8, 8)
        col = (d % 8) * 512
        return pltpu.make_async_copy(
            wqb_hbm.at[:, pl.ds(r, 8), pl.ds(col, 512)],
            wqb.at[:, pl.ds(r, 8), pl.ds(col, 512)], wsem.at[4])

    def wo_desc(src, dst, base):
        def f(s, d):
            r = pl.multiple_of((s * ND + d) * 8, 8)
            return pltpu.make_async_copy(
                src.at[:, pl.ds(r, 8)], dst.at[:, pl.ds(r, 8)], osem.at[base + s])
        return f

    wob_desc = wo_desc(wob_hbm, wob, 0)
    woa_desc = wo_desc(woa_hbm, woa, 4)

    def issue(lane0, lane1):
        for d in range(ND):
            lane0(d).start(priority=0)
            lane1(d).start(priority=1)

    def wait_all(ref, sem):
        pltpu.make_async_copy(ref, ref, sem).wait()

    def issue_pro(desc0, n0, lo=0, hi=4):
        def body(s, carry):
            issue(functools.partial(desc0, s), functools.partial(ckv_desc, n0 + s))
            return carry
        lax.fori_loop(lo, hi, body, 0)

    def issue_step(u):
        gu = u // NC
        cu = u % NC
        slot = u % NSLOT
        kd = lambda d: k_desc(gu, cu, d, slot)
        vd = lambda d: v_desc(gu - 1, cu, d, slot)

        @pl.when(jnp.logical_and(u >= NC, u < NG * NC))
        def _():
            issue(kd, vd)

        @pl.when(u < 4)
        def _():
            issue(kd, functools.partial(ckv_desc, 12 + u))

        @pl.when(jnp.logical_and(u >= 4, u < NC))
        def _():
            issue(kd, functools.partial(wuv_desc, u - 4))

        @pl.when(jnp.logical_and(u >= NG * NC, u < NG * NC + 4))
        def _():
            issue(functools.partial(wob_desc, u - NG * NC), vd)

        @pl.when(jnp.logical_and(u >= NG * NC + 4, u < (NG + 1) * NC))
        def _():
            issue(functools.partial(woa_desc, u - NG * NC - 4), vd)

    issue_pro(wqb_desc, 0, 0, 1)
    xa_cp = pltpu.make_async_copy(xa_hbm, xa, xsem.at[0])
    xb_cp = pltpu.make_async_copy(xb_hbm, xb, xsem.at[1])
    xa_cp.start()
    xb_cp.start()

    er = lax.broadcasted_iota(jnp.int32, (128, 1024), 0)
    ec = lax.broadcasted_iota(jnp.int32, (128, 1024), 1)
    for j in range(4):
        e_ref[:, j * 1024:(j + 1) * 1024] = jnp.where(
            (ec // H) + j * 32 == er, 1.0, 0.0).astype(BF16)
    ob[...] = jnp.zeros_like(ob)
    oa[...] = jnp.zeros_like(oa)
    outa[...] = jnp.zeros_like(outa)
    outb[...] = jnp.zeros_like(outb)

    issue_pro(wqb_desc, 0, 1, 4)
    issue_pro(wqa_desc, 4, 0, 2)

    xa_cp.wait()
    xb_cp.wait()
    xav = xa[...].astype(F32)
    for b in range(B):
        ya[b * H:(b + 1) * H, :] = jnp.broadcast_to(
            xav[b:b + 1, :], (H, M)).astype(BF16)
    xb8 = xb[...]

    wait_all(wqb, wsem.at[4])
    qb = jnp.dot(xb8[:, 0:128], wqb[0], preferred_element_type=F32)
    for kc in range(1, 4):
        qb += jnp.dot(xb8[:, kc * 128:(kc + 1) * 128], wqb[kc],
                      preferred_element_type=F32)
    for h in range(H):
        qb_s[pl.ds(h, B, stride=H), :] = qb[0:B, h * D:(h + 1) * D]

    issue_pro(wqa_desc, 4, 2, 4)
    issue_pro(wuk_desc, 8, 0, 4)
    for u in range(LOOK):
        issue(lambda d: k_desc(0, u, d, u % NSLOT),
              functools.partial(ckv_desc, 12 + u))

    def hmask():
        r = lax.broadcasted_iota(jnp.int32, (128, 1024), 0)
        c = lax.broadcasted_iota(jnp.int32, (128, 1024), 1)
        return (r % H) == (c % H)

    def proj_piece(w_ref, i):
        kc = i // 4
        col = pl.ds(pl.multiple_of((i % 4) * 1024, 1024), 1024)
        y = ya[:, pl.ds(pl.multiple_of(kc * 128, 128), 128)]
        lx = jnp.dot(y, e_ref[:, col], preferred_element_type=F32)
        lx = jnp.where(hmask(), lx, 0.0).astype(BF16)
        t = jnp.dot(lx, w_ref[kc, col, :], preferred_element_type=F32)

        @pl.when(i == 0)
        def _():
            pacc[...] = t

        @pl.when(i > 0)
        def _():
            pacc[...] += t

    def qabs_piece(i):
        kc = i // 4
        col = pl.ds(pl.multiple_of((i % 4) * 1024, 1024), 1024)
        gx = lax.dot_general(qa[...], wuk[kc, col, :], NT,
                             preferred_element_type=F32)
        gx = jnp.where(hmask(), gx, 0.0).astype(BF16)
        t = lax.dot_general(gx, e_ref[:, col], NT, preferred_element_type=F32)

        @pl.when(i % 4 == 0)
        def _():
            pacc[...] = t

        @pl.when(i % 4 > 0)
        def _():
            pacc[...] += t

        @pl.when(i % 4 == 3)
        def _():
            qabs[:, pl.ds(pl.multiple_of(kc * 128, 128), 128)] = (
                pacc[...].astype(BF16))

    def a_scores(b, c):
        off = pl.multiple_of(c * 1024, 1024)
        q = qabs[pl.ds(pl.multiple_of(b * H, H), H), :]
        sa[:, pl.ds(off, 1024)] = lax.dot_general(
            q, ckv[b, pl.ds(off, 1024), :], NT, preferred_element_type=F32)

    def a_softmax():
        s = sa[...]
        m = jnp.max(s, axis=1, keepdims=True)
        p = jnp.exp((s - m) * SCALE)
        pa[...] = p.astype(BF16)
        linva[...] = jnp.broadcast_to(
            1.0 / jnp.sum(p, axis=1, keepdims=True), linva.shape)

    def a_pv(b, c):
        off = pl.multiple_of(c * 1024, 1024)
        t = jnp.dot(pa[:, pl.ds(off, 1024)], ckv[b, pl.ds(off, 1024), :],
                    preferred_element_type=F32)

        @pl.when(c == 0)
        def _():
            acca[...] = t

        @pl.when(c > 0)
        def _():
            acca[...] += t

    def out_piece(o_ref, w_ref, s, regions):
        tot = None
        for r in regions:
            for jj in range(2):
                lhs = o_ref[r * HG + 2 * s + jj].astype(BF16)
                off = pl.multiple_of((2 * s + jj) * D, D)
                t = jnp.dot(lhs, w_ref[r, pl.ds(off, D), :],
                            preferred_element_type=F32)
                tot = t if tot is None else tot + t
        return tot

    def step(t, carry):
        g = t // NC
        c = t % NC
        slot = t % NSLOT
        off = pl.multiple_of(c * R, R)

        issue_step(t + LOOK)

        @pl.when(g >= 1)
        def _pv():
            wait_all(vbuf.at[slot], vsem.at[slot])
            p = p_buf[:, pl.ds(off, R)].astype(BF16)
            for j in range(HG):
                acc[j] += jnp.dot(p, vbuf[slot, j], preferred_element_type=F32)

            @pl.when(c == NC - 1)
            def _():
                gp = g - 1
                for j in range(HG):
                    o = acc[j] * linv[...]
                    ob[(gp % 4) * HG + j, pl.ds(gp // 4, 1), :] = o[j:j + 1, :]

        @pl.when(g < NG)
        def _qk():
            wait_all(kbuf.at[slot], ksem.at[slot])
            q = qb_s[pl.ds(pl.multiple_of(g * HG, HG), HG), :].astype(BF16)
            row = lax.broadcasted_iota(jnp.int32, (HG, R), 0)
            s = None
            for j in range(HG):
                r = lax.dot_general(q, kbuf[slot, j], NT,
                                    preferred_element_type=F32)
                s = r if s is None else jnp.where(row == j, r, s)
            s_buf[:, pl.ds(off, R)] = s

            @pl.when(c == NC - 1)
            def _():
                sv = s_buf[...]
                m = jnp.max(sv, axis=1, keepdims=True)
                p = jnp.exp((sv - m) * SCALE)
                p_buf[...] = p
                linv[...] = jnp.broadcast_to(
                    1.0 / jnp.sum(p, axis=1, keepdims=True), linv.shape)
                acc[...] = jnp.zeros_like(acc)

        @pl.when(t == NC)
        def _():
            wait_all(wqa, wsem.at[1])
            wait_all(wuk, wsem.at[2])
            wait_all(wuv, wsem.at[3])
            wait_all(ckv, wsem.at[0])

        @pl.when(jnp.logical_and(g >= 1, g < 3))
        def _():
            proj_piece(wqa, t - NC)

            @pl.when(t == 3 * NC - 1)
            def _():
                qa[...] = pacc[...].astype(BF16)

        @pl.when(jnp.logical_and(g >= 3, g < 5))
        def _():
            qabs_piece(t - 3 * NC)

        a_attn = jnp.logical_and(g >= 5, g < 5 + B)

        @pl.when(jnp.logical_and(a_attn, c < 4))
        def _():
            a_scores(g - 5, c)

            @pl.when(c == 3)
            def _():
                a_softmax()

        @pl.when(jnp.logical_and(a_attn, c >= 4))
        def _():
            a_pv(g - 5, c - 4)

            @pl.when(c == NC - 1)
            def _():
                li = linva[...]
                li = jnp.concatenate([li] * 4, axis=1)
                ya[pl.ds(pl.multiple_of((g - 5) * H, H), H), :] = (
                    acca[...] * li).astype(BF16)

        @pl.when(jnp.logical_and(g >= 9, g < 11))
        def _():
            proj_piece(wuv, t - 9 * NC)

            @pl.when(t == 11 * NC - 1)
            def _():
                for h in range(H):
                    oa[h, 0:B, :] = pacc[pl.ds(h, B, stride=H), :]

        @pl.when(jnp.logical_and(g == NG, c < 4))
        def _():
            rows = pl.ds(pl.multiple_of(c * 256, 256), 256)
            wait_all(wob.at[:, rows], osem.at[c])
            outb[...] += out_piece(ob, wob, c, (0, 1, 2))

        @pl.when(jnp.logical_and(g == NG, c >= 4))
        def _():
            rows = pl.ds(pl.multiple_of((c - 4) * 256, 256), 256)
            wait_all(woa.at[:, rows], osem.at[c])
            outa[...] += out_piece(oa, woa, c - 4, (0, 1, 2, 3))

        return carry

    lax.fori_loop(0, (NG + 1) * NC, step, 0)

    resb = outb[...]
    for s in range(4):
        resb += out_piece(ob, wob, s, (3,))
    resa = outa[...]
    out_ref[:, 0:M] = resa[0:B, :].astype(out_ref.dtype)
    out_ref[:, M:2 * M] = resb[0:B, :].astype(out_ref.dtype)


@jax.jit
def pallas_concat_heads__compressed_kv_cla__mha_block_cached__decode_kernel(
    A_x: jax.Array,
    A_c_kv: jax.Array,
    A_w_q: jax.Array,
    A_w_uk: jax.Array,
    A_w_uv: jax.Array,
    A_w_o: jax.Array,
    B_x: jax.Array,
    B_k_cache: jax.Array,
    B_v_cache: jax.Array,
    B_wq: jax.Array,
    B_wo: jax.Array,
):
    wqa = A_w_q.reshape(4, 128 * H, D)
    wuk = A_w_uk.reshape(4, 128 * H, D)
    wuv = A_w_uv.reshape(4, 128 * H, D)
    woa = A_w_o.reshape(4, HG * D, M)
    wqb = B_wq.reshape(4, 128, H * D)
    wob = B_wo.reshape(4, HG * D, M)

    vm = pltpu.VMEM
    scratch = [
        vm((NSLOT, HG, R, D), BF16),
        vm((NSLOT, HG, R, D), BF16),
        vm((B, SK, M), BF16),
        vm((4, 128 * H, D), BF16),
        vm((4, 128 * H, D), BF16),
        vm((4, 128 * H, D), BF16),
        vm((4, HG * D, M), BF16),
        vm((4, 128, H * D), BF16),
        vm((4, HG * D, M), BF16),
        vm((B, M), BF16),
        vm((B, M), BF16),
        vm((128, 128 * H), BF16),
        vm((B * H, D), F32),
        vm((HG, SK), F32),
        vm((HG, SK), F32),
        vm((HG, D), F32),
        vm((HG, HG, D), F32),
        vm((H, 8, D), F32),
        vm((B * H, M), BF16),
        vm((B * H, D), F32),
        vm((B * H, D), BF16),
        vm((B * H, M), BF16),
        vm((H, SK), F32),
        vm((H, SK), BF16),
        vm((H, D), F32),
        vm((H, M), F32),
        vm((H, 8, D), F32),
        vm((8, M), F32),
        vm((8, M), F32),
        pltpu.SemaphoreType.DMA((NSLOT,)),
        pltpu.SemaphoreType.DMA((NSLOT,)),
        pltpu.SemaphoreType.DMA((5,)),
        pltpu.SemaphoreType.DMA((8,)),
        pltpu.SemaphoreType.DMA((2,)),
    ]
    out = pl.pallas_call(
        _kernel,
        in_specs=[pl.BlockSpec(memory_space=pl.ANY)] * 11,
        out_specs=pl.BlockSpec(memory_space=pltpu.VMEM),
        out_shape=jax.ShapeDtypeStruct((B, 2 * M), A_x.dtype),
        scratch_shapes=scratch,
        compiler_params=pltpu.CompilerParams(
            vmem_limit_bytes=96 * 1024 * 1024),
    )(A_x.reshape(B, M), A_c_kv, wqa, wuk, wuv, woa, B_x.reshape(B, M),
      B_k_cache, B_v_cache, wqb, wob)
    return out.reshape(B, 1, 2 * M)
```

```python
import jax
import jax.numpy as jnp
from jax import lax
import jax.experimental.pallas as pl
import jax.experimental.pallas.tpu as pltpu

F32 = jnp.float32
BF16 = jnp.bfloat16

B = 4
H = 32
SK = 4096
D = 128
M = 512
HG = 8
NG = B * H // HG
R = 512
NC = SK // R
NSTEP = NG * NC
HOFF = 2
WRAP = HG - HOFF
LOOK = 2
VLAG = 6
KS = LOOK + 1
VS = LOOK + 1 + NC - VLAG
A0 = 16
SCALE = float(D) ** -0.5

NT = (((1,), (1,)), ((), ()))

_sizes = [24] + [16] * 30 + [8]
KV_ROWS = [(sum(_sizes[:i]), s) for i, s in enumerate(_sizes)]


def _merge(a, b):
    out, ia, ib, ca, cb = [], 0, 0, 0, 0
    while ia < len(a) or ib < len(b):
        if ib >= len(b) or (ia < len(a) and ca <= cb):
            out.append((0, a[ia][1]))
            ca += a[ia][0]
            ia += 1
        else:
            out.append((1, b[ib][1]))
            cb += b[ib][0]
            ib += 1
    return out


def _kernel(
    xa_hbm, ckv_hbm, wqa_hbm, wuk_hbm, wuv_hbm, woa_hbm,
    xb_hbm, k_hbm, v_hbm, wqb_hbm, wob_hbm,
    out_ref,
    kbuf, vbuf, ckv, wqa, wuk, wuv, woa, wqb, wob, xa, xb,
    e_ref, qb_s, s_buf, p_buf, linv, acc, ob,
    ya, pacc, qa, qabs, sa, pa, linva, acca, oa,
    ksem, vsem, wsem, osem, xsem,
):
    cp = pltpu.make_async_copy

    def kv_step(src, dst, sem, g, c):
        h0 = g * HG - WRAP
        r0 = c * R
        return [(n, cp(src.at[pl.ds(h0, HG), pl.ds(pl.multiple_of(r0 + o, 8), n)],
                       dst.at[:, pl.ds(o, n)], sem)) for o, n in KV_ROWS]

    def kv_wrap_step(src, dst, sem, c):
        r0 = c * R
        out = []
        for i, (o, n) in enumerate(KV_ROWS):
            out.append((n * WRAP / HG, cp(
                src.at[pl.ds(B * H - WRAP, WRAP), pl.ds(pl.multiple_of(r0 + o, 8), n)],
                dst.at[pl.ds(0, WRAP), pl.ds(o, n)], sem)))
            if HOFF and i % 4 == 3:
                o2 = (i // 4) * 64
                out.append((64 * HOFF / HG, cp(
                    src.at[pl.ds(0, HOFF), pl.ds(pl.multiple_of(r0 + o2, 8), 64)],
                    dst.at[pl.ds(WRAP, HOFF), pl.ds(o2, 64)], sem)))
        return out

    def k_step(u, wrap):
        slot = u % KS
        if wrap:
            return kv_wrap_step(k_hbm, kbuf.at[slot], ksem.at[slot], u % NC)
        return kv_step(k_hbm, kbuf.at[slot], ksem.at[slot], u // NC, u % NC)

    def v_step(u, wrap):
        w = u - VLAG
        slot = w % VS
        if wrap:
            return kv_wrap_step(v_hbm, vbuf.at[slot], vsem.at[slot], u % NC)
        return kv_step(v_hbm, vbuf.at[slot], vsem.at[slot], w // NC, u % NC)

    def wide_step(src, dst, sem, s):
        out = []
        for d in range(32):
            idx = (slice(None), pl.ds(pl.multiple_of(s * 128 + (d // 2) * 8, 8), 8),
                   pl.ds((d % 2) * 256, 256))
            out.append((16, cp(src.at[idx], dst.at[idx], sem)))
        return out

    def w3_step(src, dst, sem, s):
        out = []
        for d in range(32):
            idx = (slice(None), pl.ds(pl.multiple_of(s * 512 + d * 16, 16), 16))
            out.append((16, cp(src.at[idx], dst.at[idx], sem)))
        return out

    def wqb_step(s):
        out = []
        for d in range(32):
            idx = (slice(None), pl.ds(pl.multiple_of(s * 16 + (d // 16) * 8, 8), 8),
                   pl.ds((d % 16) * 256, 256))
            out.append((16, cp(wqb_hbm.at[idx], wqb.at[idx], wsem.at[4])))
        return out

    ckv_step = lambda s: wide_step(ckv_hbm, ckv, wsem.at[0], s)
    wqa_step = lambda s: w3_step(wqa_hbm, wqa, wsem.at[1], s)
    wuk_step = lambda s: w3_step(wuk_hbm, wuk, wsem.at[2], s)
    wuv_step = lambda s: w3_step(wuv_hbm, wuv, wsem.at[3], s)
    wob_step = lambda s: wide_step(wob_hbm, wob, osem.at[s], s)
    woa_step = lambda s: wide_step(woa_hbm, woa, osem.at[4 + s], s)

    def woa_tail(lane):
        out = []
        for r in range(3 * lane, 3 * lane + 3):
            for o in range(256, 512, 32):
                idx = (r, pl.ds(o, 32))
                out.append((16, cp(woa_hbm.at[idx], woa.at[idx], osem.at[6])))
        for o in range(256, 512, 32):
            idx = (6 + lane, pl.ds(o, 32))
            out.append((16, cp(woa_hbm.at[idx], woa.at[idx],
                               osem.at[7 if o < 384 else 8])))
        return out

    def issue(lane0, lane1):
        for lane, c in _merge(lane0, lane1):
            c.start(priority=lane)

    def wait_all(ref, sem):
        cp(ref, ref, sem).wait()

    def issue_pro(step0, n0, lo, hi):
        def body(s, carry):
            issue(step0(s), ckv_step(n0 + s))
            return carry
        lax.fori_loop(lo, hi, body, 0)

    variants = [
        (0, 3, lambda u: (k_step(u, True), ckv_step(13 + u))),
        (3, VLAG, lambda u: (k_step(u, True), wuv_step(u - 2))),
        (VLAG, NC, lambda u: (k_step(u, True), v_step(u, True))),
        (NC, NC + VLAG, lambda u: (k_step(u, False), v_step(u, True))),
        (NC + VLAG, NSTEP, lambda u: (k_step(u, False), v_step(u, False))),
        (NSTEP, NSTEP + 4, lambda u: (wob_step(u - NSTEP), v_step(u, False))),
        (NSTEP + 4, NSTEP + 6,
         lambda u: (woa_step(u - NSTEP - 4), v_step(u, False))),
        (NSTEP + 6, NSTEP + 7, lambda u: (woa_tail(0), woa_tail(1))),
    ]

    def issue_static(u):
        for lo, hi, f in variants:
            if lo <= u < hi:
                issue(*f(u))

    def issue_dynamic(u, umin, umax):
        for lo, hi, f in sorted(variants, key=lambda v: v[0] - v[1]):
            if hi > umin and lo <= umax:
                pl.when(jnp.logical_and(u >= lo, u < hi))(
                    lambda f=f: issue(*f(u)))

    issue(wqb_step(0), ckv_step(0))
    xa_cp = cp(xa_hbm, xa, xsem.at[0])
    xb_cp = cp(xb_hbm, xb, xsem.at[1])
    xa_cp.start()
    xb_cp.start(priority=1)

    er = lax.broadcasted_iota(jnp.int32, (128, 1024), 0)
    ec = lax.broadcasted_iota(jnp.int32, (128, 1024), 1)
    for j in range(4):
        e_ref[:, j * 1024:(j + 1) * 1024] = jnp.where(
            (ec // H) + j * 32 == er, 1.0, 0.0).astype(BF16)
    ob[...] = jnp.zeros_like(ob)
    oa[...] = jnp.zeros_like(oa)

    issue_pro(wqb_step, 0, 1, 4)
    issue_pro(wqa_step, 4, 0, 2)

    xa_cp.wait()
    xb_cp.wait()
    xav = xa[...].astype(F32)
    for b in range(B):
        ya[b * H:(b + 1) * H, :] = jnp.broadcast_to(
            xav[b:b + 1, :], (H, M)).astype(BF16)
    xbv = xb[...]

    wait_all(wqb, wsem.at[4])
    qb = None
    for kc in range(4):
        w = wqb[2 * kc:2 * kc + 2].reshape(128, H * D)
        t = jnp.dot(xbv[:, kc * 128:(kc + 1) * 128], w,
                    preferred_element_type=F32)
        qb = t if qb is None else qb + t
    for h in range(H):
        col = qb[:, h * D:(h + 1) * D]
        if h + WRAP < H:
            qb_s[pl.ds(h + WRAP, B, stride=H), :] = col
        else:
            qb_s[pl.ds(h + WRAP, B - 1, stride=H), :] = col[0:B - 1]
            qb_s[pl.ds(h + WRAP - H, 1), :] = col[B - 1:B]

    issue_pro(wqa_step, 4, 2, 4)
    issue_pro(wuk_step, 8, 0, 4)
    issue(wuv_step(0), ckv_step(12))
    for u in range(LOOK):
        issue_static(u)

    def hmask():
        r = lax.broadcasted_iota(jnp.int32, (128, 1024), 0)
        c = lax.broadcasted_iota(jnp.int32, (128, 1024), 1)
        return (r % H) == (c % H)

    def w_piece(w_ref, i):
        return w_ref[i // 2, pl.ds(pl.multiple_of((i % 2) * 1024, 1024), 1024), :]

    def e_piece(i):
        return e_ref[:, pl.ds(pl.multiple_of((i % 4) * 1024, 1024), 1024)]

    def accumulate(ref, t, first):
        @pl.when(first)
        def _():
            ref[...] = t

        @pl.when(jnp.logical_not(first))
        def _():
            ref[...] += t

    def proj_piece(w_ref, i):
        y = ya[:, pl.ds(pl.multiple_of((i // 4) * 128, 128), 128)]
        lx = jnp.dot(y, e_piece(i), preferred_element_type=F32)
        lx = jnp.where(hmask(), lx, 0.0).astype(BF16)
        accumulate(pacc, jnp.dot(lx, w_piece(w_ref, i),
                                 preferred_element_type=F32), i == 0)

    def qabs_piece(i):
        gx = lax.dot_general(qa[...], w_piece(wuk, i), NT,
                             preferred_element_type=F32)
        gx = jnp.where(hmask(), gx, 0.0).astype(BF16)
        accumulate(pacc, lax.dot_general(gx, e_piece(i), NT,
                                         preferred_element_type=F32), i % 4 == 0)

        @pl.when(i % 4 == 3)
        def _():
            qabs[:, pl.ds(pl.multiple_of((i // 4) * 128, 128), 128)] = (
                pacc[...].astype(BF16))

    def ckv_piece(b, c):
        return ckv[2 * b + c // 2,
                   pl.ds(pl.multiple_of((c % 2) * 1024, 1024), 1024), :]

    def a_scores(b, c):
        q = qabs[pl.ds(pl.multiple_of(b * H, H), H), :]
        sa[:, pl.ds(pl.multiple_of(c * 1024, 1024), 1024)] = lax.dot_general(
            q, ckv_piece(b, c), NT, preferred_element_type=F32)

    def softmax(s_ref, p_ref, linv_ref):
        s = s_ref[...]
        m = jnp.max(s, axis=1, keepdims=True)
        p = jnp.exp((s - m) * SCALE)
        p_ref[...] = p.astype(p_ref.dtype)
        linv_ref[...] = jnp.broadcast_to(
            1.0 / jnp.sum(p, axis=1, keepdims=True), linv_ref.shape)

    def a_pv(b, c):
        p = pa[:, pl.ds(pl.multiple_of(c * 1024, 1024), 1024)]
        accumulate(acca, jnp.dot(p, ckv_piece(b, c),
                                 preferred_element_type=F32), c == 0)

    def a_piece(i):
        @pl.when(i == 0)
        def _():
            wait_all(wqa, wsem.at[1])
            wait_all(wuk, wsem.at[2])
            wait_all(wuv, wsem.at[3])
            wait_all(ckv, wsem.at[0])

        @pl.when(i < 16)
        def _():
            proj_piece(wqa, i)

            @pl.when(i == 15)
            def _():
                qa[...] = pacc[...].astype(BF16)

        @pl.when(jnp.logical_and(i >= 16, i < 32))
        def _():
            qabs_piece(i - 16)

        attn = jnp.logical_and(i >= 32, i < 64)
        b = (i - 32) // 8
        c = i % 8

        @pl.when(jnp.logical_and(attn, c < 4))
        def _():
            a_scores(b, c)

            @pl.when(c == 3)
            def _():
                softmax(sa, pa, linva)

        @pl.when(jnp.logical_and(attn, c >= 4))
        def _():
            a_pv(b, c - 4)

            @pl.when(c == 7)
            def _():
                li = jnp.concatenate([linva[...]] * 4, axis=1)
                ya[pl.ds(pl.multiple_of(b * H, H), H), :] = (
                    acca[...] * li).astype(BF16)

        @pl.when(i >= 64)
        def _():
            proj_piece(wuv, i - 64)

            @pl.when(i == 79)
            def _():
                for h in range(H):
                    oa[h, 0:B, :] = pacc[pl.ds(h, B, stride=H), :]

    def pv(w):
        slot = w % VS
        wait_all(vbuf.at[slot], vsem.at[slot])
        off = ((w + VLAG) % NC) * R
        if not isinstance(off, int):
            off = pl.multiple_of(off, R)
        p = p_buf[:, pl.ds(off, R)].astype(BF16)
        for j in range(HG):
            acc[j] += jnp.dot(p, vbuf[slot, j], preferred_element_type=F32)

    def finish_group(g):
        for j in range(HG):
            n = (g * HG + (B * H - WRAP + j)) % (B * H)
            o = acc[j] * linv[...]
            ob[n % H, pl.ds(n // H, 1), :] = o[j:j + 1, :]

    def qk(t):
        slot = t % KS
        wait_all(kbuf.at[slot], ksem.at[slot])
        q = qb_s[pl.ds(pl.multiple_of((t // NC) * HG, HG), HG), :].astype(BF16)
        row = lax.broadcasted_iota(jnp.int32, (HG, R), 0)
        s = None
        for j in range(HG):
            r = lax.dot_general(q, kbuf[slot, j], NT, preferred_element_type=F32)
            s = r if s is None else jnp.where(row == j, r, s)
        s_buf[:, pl.ds(pl.multiple_of((t % NC) * R, R), R)] = s

    def out_proj(o_ref, w_ref, heads, tot):
        for h in heads:
            t = jnp.dot(o_ref[h].astype(BF16),
                        w_ref[h // 4, (h % 4) * D:(h % 4 + 1) * D, :],
                        preferred_element_type=F32)
            tot = t if tot is None else tot + t
        return tot

    def step(t, carry):
        issue_dynamic(t + LOOK, LOOK, NSTEP - 1 + LOOK)
        last = t % NC == NC - 1

        @pl.when(t >= NC)
        def _():
            pv(t - NC)

            @pl.when(last)
            def _():
                finish_group(t // NC - 1)

        qk(t)

        @pl.when(last)
        def _():
            softmax(s_buf, p_buf, linv)
            acc[...] = jnp.zeros_like(acc)

        @pl.when(jnp.logical_and(t >= A0, t < A0 + 80))
        def _():
            a_piece(t - A0)

        return carry

    lax.fori_loop(0, NSTEP, step, 0)

    late = [((NG - 1) * HG - WRAP + j) % H for j in range(HG)]
    resa = resb = None
    w = NSTEP - NC
    for t in range(NSTEP, NSTEP + VLAG):
        issue_static(t + LOOK)
        while w <= t - VLAG:
            pv(w)
            w += 1
        s = t - NSTEP
        if s == VLAG - 1:
            finish_group(NG - 1)
            resb = out_proj(ob, wob, late, resb)
            out_ref[:, M:2 * M] = resb[0:B, :].astype(out_ref.dtype)
        if s < 4:
            wait_all(wob.at[:, pl.ds(s * 128, 128)], osem.at[s])
            resb = out_proj(ob, wob, [h for h in range(s, H, 4) if h not in late],
                            resb)
        else:
            wait_all(woa.at[:, pl.ds((s - 4) * 128, 128)], osem.at[s])
            resa = out_proj(oa, woa, range(s - 4, H, 4), resa)

    wait_all(woa.at[pl.ds(0, 6), pl.ds(256, 256)], osem.at[6])
    resa = out_proj(oa, woa, [4 * r + s for r in range(6) for s in (2, 3)], resa)
    wait_all(woa.at[pl.ds(6, 2), pl.ds(256, 128)], osem.at[7])
    resa = out_proj(oa, woa, [26, 30], resa)
    wait_all(woa.at[pl.ds(6, 2), pl.ds(384, 128)], osem.at[8])
    resa = out_proj(oa, woa, [27, 31], resa)
    out_ref[:, 0:M] = resa[0:B, :].astype(out_ref.dtype)


@jax.jit
def pallas_concat_heads__compressed_kv_cla__mha_block_cached__decode_kernel(
    A_x: jax.Array,
    A_c_kv: jax.Array,
    A_w_q: jax.Array,
    A_w_uk: jax.Array,
    A_w_uv: jax.Array,
    A_w_o: jax.Array,
    B_x: jax.Array,
    B_k_cache: jax.Array,
    B_v_cache: jax.Array,
    B_wq: jax.Array,
    B_wo: jax.Array,
):
    args = (
        A_x.reshape(B, M),
        A_c_kv.reshape(8, SK // 2, M),
        A_w_q.reshape(8, 64 * H, D),
        A_w_uk.reshape(8, 64 * H, D),
        A_w_uv.reshape(8, 64 * H, D),
        A_w_o.reshape(8, 4 * D, M),
        B_x.reshape(B, M),
        B_k_cache.reshape(B * H, SK, D),
        B_v_cache.reshape(B * H, SK, D),
        B_wq.reshape(8, 64, H * D),
        B_wo.reshape(8, 4 * D, M),
    )

    vm = pltpu.VMEM
    scratch = [
        vm((KS, HG, R, D), BF16),
        vm((VS, HG, R, D), BF16),
        vm((8, SK // 2, M), BF16),
        vm((8, 64 * H, D), BF16),
        vm((8, 64 * H, D), BF16),
        vm((8, 64 * H, D), BF16),
        vm((8, 4 * D, M), BF16),
        vm((8, 64, H * D), BF16),
        vm((8, 4 * D, M), BF16),
        vm((B, M), BF16),
        vm((B, M), BF16),
        vm((128, 128 * H), BF16),
        vm((B * H, D), F32),
        vm((HG, SK), F32),
        vm((HG, SK), F32),
        vm((HG, D), F32),
        vm((HG, HG, D), F32),
        vm((H, 8, D), F32),
        vm((B * H, M), BF16),
        vm((B * H, D), F32),
        vm((B * H, D), BF16),
        vm((B * H, M), BF16),
        vm((H, SK), F32),
        vm((H, SK), BF16),
        vm((H, D), F32),
        vm((H, M), F32),
        vm((H, 8, D), F32),
        pltpu.SemaphoreType.DMA((KS,)),
        pltpu.SemaphoreType.DMA((VS,)),
        pltpu.SemaphoreType.DMA((5,)),
        pltpu.SemaphoreType.DMA((9,)),
        pltpu.SemaphoreType.DMA((2,)),
    ]
    out = pl.pallas_call(
        _kernel,
        in_specs=[pl.BlockSpec(memory_space=pl.ANY)] * 11,
        out_specs=pl.BlockSpec(memory_space=pltpu.VMEM),
        out_shape=jax.ShapeDtypeStruct((B, 2 * M), A_x.dtype),
        scratch_shapes=scratch,
        compiler_params=pltpu.CompilerParams(
            vmem_limit_bytes=96 * 1024 * 1024,
            disable_bounds_checks=True),
    )(*args)
    return out.reshape(B, 1, 2 * M)
```

```python
import jax
import jax.numpy as jnp
from jax import lax
import jax.experimental.pallas as pl
import jax.experimental.pallas.tpu as pltpu

F32 = jnp.float32
BF16 = jnp.bfloat16

B = 4
H = 32
SK = 4096
D = 128
M = 512
HG = 8
NG = B * H // HG
R = 512
NC = SK // R
NSTEP = NG * NC
LOOK = 2
VLAG = 6
KS = LOOK + 1
VS = LOOK + 1 + NC - VLAG
A0 = 16
SCALE = float(D) ** -0.5

NT = (((1,), (1,)), ((), ()))

PHA = 15
PHB = 17
SW = 4
SC = 8


def _pieces(width, t0, t1):
    per = width // 128
    out = []
    while t0 < t1:
        s, c = divmod(t0, per)
        if c == 0 and t1 - t0 >= per:
            n = (t1 - t0) // per
            out.append((pl.ds(s * 8, n * 8), pl.ds(0, width)))
            t0 += n * per
        else:
            e = min(t1, (s + 1) * per)
            out.append((pl.ds(s * 8, 8), pl.ds(c * 128, (e - t0) * 128)))
            t0 = e
    return out


TAIL = [(0, 4, 2), (4, 4, 2), (0, 4, 3), (4, 2, 3), (6, 2, 3)]


def _kernel(
    xa_hbm, ckv_hbm, wqa_hbm, wuk_hbm, wuv_hbm, woa_hbm,
    xb_hbm, k_hbm, v_hbm, wqb_hbm, wob_hbm,
    out_ref,
    kbuf, vbuf, ckv, wqa, wuk, wuv, woa, wqb, wob, xa, xb,
    e_ref, qb_s, s_buf, p_buf, linv, acc, ob,
    ya, pacc, qa, qabs, sa, pa, linva, acca, oa,
    ksem, vsem, wsem, osem, xsem,
):
    cp = pltpu.make_async_copy

    def part(src, dst, lo, ph, sem):
        w = src.shape[-1]
        rects = _pieces(w, 0, ph) if lo else _pieces(w, ph, 32)
        return [cp(src.at[r], dst.at[r], sem) for r in rects]

    def kv_step(src, dst, sem, g, c):
        out = []
        wrap = (c + 1) // NC
        for u in range(2):
            for j in range(HG):
                k = j * 16 + 2 * c + u
                jn = j if u == 0 else (j + wrap) % HG
                kn = k + 1 if j < HG - 1 or u == 0 else (k + 1) % 128
                out.append(part(src.at[g * 128 + k], dst.at[j, u], False, PHB, sem))
                out.append(part(src.at[g * 128 + kn], dst.at[jn, u], True, PHB, sem))
        return out

    def k_step(u):
        slot = u % KS
        return kv_step(k_hbm, kbuf.at[slot], ksem.at[slot], u // NC, u % NC)

    def v_step(u):
        w = u - VLAG
        slot = w % VS
        return kv_step(v_hbm, vbuf.at[slot], vsem.at[slot], w // NC, u % NC)

    def ring_step(src, dst, sem, ph, ns):
        nb = src.shape[0]
        nv = 16 // ns

        def f(s):
            out = []
            for i in range(nv):
                for r in range(ns):
                    k = r * (nb // ns) + s * nv + i
                    kn = (k + 1) % nb if r == ns - 1 and i == nv - 1 else k + 1
                    out.append(part(src.at[k], dst.at[k], False, ph, sem))
                    out.append(part(src.at[kn], dst.at[kn], True, ph, sem))
            return out
        return f

    ckv_step = ring_step(ckv_hbm, ckv, wsem.at[0], PHA, SC)
    wqa_step = ring_step(wqa_hbm, wqa, wsem.at[1], PHA, SW)
    wuk_step = ring_step(wuk_hbm, wuk, wsem.at[2], PHA, SW)
    wuv_step = ring_step(wuv_hbm, wuv, wsem.at[3], PHA, SW)
    wqb_step = ring_step(wqb_hbm, wqb, wsem.at[4], PHB, SW)

    def wo_heads(src, dst, ph, semf, regions, hh):
        out = []
        if hh == 0:
            out += [part(src.at[r, 0], dst.at[r, 0], True, ph, semf(r, 0))
                    for r in regions]
        for k in (2 * hh, 2 * hh + 1):
            for r in regions:
                out.append(part(src.at[r, k], dst.at[r, k], False, ph, semf(r, hh)))
                if k < 7:
                    out.append(part(src.at[r, k + 1], dst.at[r, k + 1], True, ph,
                                    semf(r, (k + 1) // 2)))
        return out

    def woa_sem(r, hh):
        if hh < 2:
            return osem.at[4 + hh]
        i, = [i for i, (r0, nr, h) in enumerate(TAIL)
              if h == hh and r0 <= r < r0 + nr]
        return osem.at[6 + i]

    wob_step = lambda s: wo_heads(wob_hbm, wob, PHB, lambda r, hh: osem.at[hh],
                                  range(8), s)
    woa_step = lambda s: wo_heads(woa_hbm, woa, PHA, woa_sem, range(8), s)

    def woa_tail(lane):
        out = []
        for r0, nr, hh in TAIL:
            h = nr // 2
            out += wo_heads(woa_hbm, woa, PHA, woa_sem,
                            range(r0 + lane * h, r0 + (lane + 1) * h), hh)
        return out

    def issue(lane0, lane1):
        for i in range(max(len(lane0), len(lane1))):
            for lane, slots in enumerate((lane0, lane1)):
                if i < len(slots):
                    for c in slots[i]:
                        c.start(priority=lane)

    def wait_all(ref, sem):
        cp(ref, ref, sem).wait()

    def issue_pro(step0, n0, lo, hi):
        def body(s, carry):
            issue(step0(s), ckv_step(n0 + s))
            return carry
        lax.fori_loop(lo, hi, body, 0)

    variants = [
        (0, 3, lambda u: (k_step(u), ckv_step(13 + u))),
        (3, VLAG, lambda u: (k_step(u), wuv_step(u - 2))),
        (VLAG, NSTEP, lambda u: (k_step(u), v_step(u))),
    ] + [
        (NSTEP + s, NSTEP + s + 1,
         lambda u, s=s: (wob_step(s) if s < 4 else woa_step(s - 4),
                         v_step(NSTEP + s)))
        for s in range(VLAG)
    ] + [
        (NSTEP + VLAG, NSTEP + VLAG + 1, lambda u: (woa_tail(0), woa_tail(1))),
    ]

    def issue_static(u):
        for lo, hi, f in variants:
            if lo <= u < hi:
                issue(*f(u))

    def issue_dynamic(u, umin, umax):
        for lo, hi, f in sorted(variants, key=lambda v: v[0] - v[1]):
            if hi > umin and lo <= umax:
                pl.when(jnp.logical_and(u >= lo, u < hi))(
                    lambda f=f: issue(*f(u)))

    issue(wqb_step(0), ckv_step(0))
    xa_cp = cp(xa_hbm, xa, xsem.at[0])
    xb_cp = cp(xb_hbm, xb, xsem.at[1])
    xa_cp.start()
    xb_cp.start(priority=1)

    er = lax.broadcasted_iota(jnp.int32, (128, 1024), 0)
    ec = lax.broadcasted_iota(jnp.int32, (128, 1024), 1)
    for j in range(4):
        e_ref[:, j * 1024:(j + 1) * 1024] = jnp.where(
            (ec // H) + j * 32 == er, 1.0, 0.0).astype(BF16)
    ob[...] = jnp.zeros_like(ob)
    oa[...] = jnp.zeros_like(oa)

    issue_pro(wqb_step, 0, 1, 4)
    issue_pro(wqa_step, 4, 0, 2)

    xa_cp.wait()
    xb_cp.wait()
    xav = xa[...].astype(F32)
    for b in range(B):
        ya[b * H:(b + 1) * H, :] = jnp.broadcast_to(
            xav[b:b + 1, :], (H, M)).astype(BF16)
    xbv = xb[...]

    wait_all(wqb, wsem.at[4])
    qb = None
    for kc in range(4):
        w = wqb[16 * kc:16 * kc + 16].reshape(128, H * D)
        t = jnp.dot(xbv[:, kc * 128:(kc + 1) * 128], w,
                    preferred_element_type=F32)
        qb = t if qb is None else qb + t
    for h in range(H):
        qb_s[pl.ds(h, B, stride=H), :] = qb[:, h * D:(h + 1) * D]

    issue_pro(wqa_step, 4, 2, 4)
    issue_pro(wuk_step, 8, 0, 4)
    issue(wuv_step(0), ckv_step(12))
    for u in range(LOOK):
        issue_static(u)

    def hmask():
        r = lax.broadcasted_iota(jnp.int32, (128, 1024), 0)
        c = lax.broadcasted_iota(jnp.int32, (128, 1024), 1)
        return (r % H) == (c % H)

    def w_piece(w_ref, i):
        return w_ref[pl.ds(i * 4, 4)].reshape(1024, D)

    def e_piece(i):
        return e_ref[:, pl.ds(pl.multiple_of((i % 4) * 1024, 1024), 1024)]

    def accumulate(ref, t, first):
        @pl.when(first)
        def _():
            ref[...] = t

        @pl.when(jnp.logical_not(first))
        def _():
            ref[...] += t

    def proj_piece(w_ref, i):
        y = ya[:, pl.ds(pl.multiple_of((i // 4) * 128, 128), 128)]
        lx = jnp.dot(y, e_piece(i), preferred_element_type=F32)
        lx = jnp.where(hmask(), lx, 0.0).astype(BF16)
        accumulate(pacc, jnp.dot(lx, w_piece(w_ref, i),
                                 preferred_element_type=F32), i == 0)

    def qabs_piece(i):
        gx = lax.dot_general(qa[...], w_piece(wuk, i), NT,
                             preferred_element_type=F32)
        gx = jnp.where(hmask(), gx, 0.0).astype(BF16)
        accumulate(pacc, lax.dot_general(gx, e_piece(i), NT,
                                         preferred_element_type=F32), i % 4 == 0)

        @pl.when(i % 4 == 3)
        def _():
            qabs[:, pl.ds(pl.multiple_of((i // 4) * 128, 128), 128)] = (
                pacc[...].astype(BF16))

    def ckv_piece(b, c):
        return ckv[pl.ds((b * 4 + c) * 16, 16)].reshape(1024, M)

    def a_scores(b, c):
        q = qabs[pl.ds(pl.multiple_of(b * H, H), H), :]
        sa[:, pl.ds(pl.multiple_of(c * 1024, 1024), 1024)] = lax.dot_general(
            q, ckv_piece(b, c), NT, preferred_element_type=F32)

    def softmax(s_ref, p_ref, linv_ref):
        s = s_ref[...]
        m = jnp.max(s, axis=1, keepdims=True)
        p = jnp.exp((s - m) * SCALE)
        p_ref[...] = p.astype(p_ref.dtype)
        linv_ref[...] = jnp.broadcast_to(
            1.0 / jnp.sum(p, axis=1, keepdims=True), linv_ref.shape)

    def a_pv(b, c):
        p = pa[:, pl.ds(pl.multiple_of(c * 1024, 1024), 1024)]
        accumulate(acca, jnp.dot(p, ckv_piece(b, c),
                                 preferred_element_type=F32), c == 0)

    def a_piece(i):
        @pl.when(i == 0)
        def _():
            wait_all(wqa, wsem.at[1])
            wait_all(wuk, wsem.at[2])
            wait_all(wuv, wsem.at[3])
            wait_all(ckv, wsem.at[0])

        @pl.when(i < 16)
        def _():
            proj_piece(wqa, i)

            @pl.when(i == 15)
            def _():
                qa[...] = pacc[...].astype(BF16)

        @pl.when(jnp.logical_and(i >= 16, i < 32))
        def _():
            qabs_piece(i - 16)

        attn = jnp.logical_and(i >= 32, i < 64)
        b = (i - 32) // 8
        c = i % 8

        @pl.when(jnp.logical_and(attn, c < 4))
        def _():
            a_scores(b, c)

            @pl.when(c == 3)
            def _():
                softmax(sa, pa, linva)

        @pl.when(jnp.logical_and(attn, c >= 4))
        def _():
            a_pv(b, c - 4)

            @pl.when(c == 7)
            def _():
                li = jnp.concatenate([linva[...]] * 4, axis=1)
                ya[pl.ds(pl.multiple_of(b * H, H), H), :] = (
                    acca[...] * li).astype(BF16)

        @pl.when(i >= 64)
        def _():
            proj_piece(wuv, i - 64)

            @pl.when(i == 79)
            def _():
                for h in range(H):
                    oa[h, 0:B, :] = pacc[pl.ds(h, B, stride=H), :]

    def pv(w):
        slot = w % VS
        wait_all(vbuf.at[slot], vsem.at[slot])
        off = ((w + VLAG) % NC) * R
        if not isinstance(off, int):
            off = pl.multiple_of(off, R)
        p = p_buf[:, pl.ds(off, R)].astype(BF16)
        for j in range(HG):
            acc[j] += jnp.dot(p, vbuf[slot, j].reshape(R, D),
                              preferred_element_type=F32)

    def finish_group(g):
        for j in range(HG):
            o = acc[j] * linv[...]
            ob[(g % 4) * HG + j, pl.ds(g // 4, 1), :] = o[j:j + 1, :]

    def qk(t):
        slot = t % KS
        wait_all(kbuf.at[slot], ksem.at[slot])
        q = qb_s[pl.ds(pl.multiple_of((t // NC) * HG, HG), HG), :].astype(BF16)
        row = lax.broadcasted_iota(jnp.int32, (HG, R), 0)
        s = None
        for j in range(HG):
            r = lax.dot_general(q, kbuf[slot, j].reshape(R, D), NT,
                                preferred_element_type=F32)
            s = r if s is None else jnp.where(row == j, r, s)
        s_buf[:, pl.ds(pl.multiple_of((t % NC) * R, R), R)] = s

    def out_proj(o_ref, w_ref, heads, tot):
        for h in heads:
            t = jnp.dot(o_ref[h].astype(BF16),
                        w_ref[h // 4, 2 * (h % 4):2 * (h % 4) + 2].reshape(D, M),
                        preferred_element_type=F32)
            tot = t if tot is None else tot + t
        return tot

    def step(t, carry):
        issue_dynamic(t + LOOK, LOOK, NSTEP - 1 + LOOK)
        last = t % NC == NC - 1

        @pl.when(t >= NC)
        def _():
            pv(t - NC)

            @pl.when(last)
            def _():
                finish_group(t // NC - 1)

        qk(t)

        @pl.when(last)
        def _():
            softmax(s_buf, p_buf, linv)
            acc[...] = jnp.zeros_like(acc)

        @pl.when(jnp.logical_and(t >= A0, t < A0 + 80))
        def _():
            a_piece(t - A0)

        return carry

    lax.fori_loop(0, NSTEP, step, 0)

    late = range(H - HG, H)
    resa = resb = None
    w = NSTEP - NC
    for t in range(NSTEP, NSTEP + VLAG):
        issue_static(t + LOOK)
        while w <= t - VLAG:
            pv(w)
            w += 1
        s = t - NSTEP
        if s == VLAG - 1:
            finish_group(NG - 1)
            resb = out_proj(ob, wob, late, resb)
            out_ref[:, M:2 * M] = resb[0:B, :].astype(out_ref.dtype)
        if s < 4:
            wait_all(wob.at[:, pl.ds(2 * s, 2)], osem.at[s])
            resb = out_proj(ob, wob, [h for h in range(s, H, 4) if h not in late],
                            resb)
        else:
            wait_all(woa.at[:, pl.ds(2 * (s - 4), 2)], osem.at[s])
            resa = out_proj(oa, woa, range(s - 4, H, 4), resa)

    for i, (r0, nr, hh) in enumerate(TAIL):
        wait_all(woa.at[pl.ds(r0, nr), pl.ds(2 * hh, 2)], osem.at[6 + i])
        resa = out_proj(oa, woa, [4 * r + hh for r in range(r0, r0 + nr)], resa)
    out_ref[:, 0:M] = resa[0:B, :].astype(out_ref.dtype)


@jax.jit
def pallas_concat_heads__compressed_kv_cla__mha_block_cached__decode_kernel(
    A_x: jax.Array,
    A_c_kv: jax.Array,
    A_w_q: jax.Array,
    A_w_uk: jax.Array,
    A_w_uv: jax.Array,
    A_w_o: jax.Array,
    B_x: jax.Array,
    B_k_cache: jax.Array,
    B_v_cache: jax.Array,
    B_wq: jax.Array,
    B_wo: jax.Array,
):
    args = (
        A_x.reshape(B, M),
        A_c_kv.reshape(256, 64, M),
        A_w_q.reshape(64, 256, D),
        A_w_uk.reshape(64, 256, D),
        A_w_uv.reshape(64, 256, D),
        A_w_o.reshape(8, 8, 64, M),
        B_x.reshape(B, M),
        B_k_cache.reshape(2048, 256, D),
        B_v_cache.reshape(2048, 256, D),
        B_wq.reshape(64, 8, H * D),
        B_wo.reshape(8, 8, 64, M),
    )

    vm = pltpu.VMEM
    scratch = [
        vm((KS, HG, 2, 256, D), BF16),
        vm((VS, HG, 2, 256, D), BF16),
        vm((256, 64, M), BF16),
        vm((64, 256, D), BF16),
        vm((64, 256, D), BF16),
        vm((64, 256, D), BF16),
        vm((8, 8, 64, M), BF16),
        vm((64, 8, H * D), BF16),
        vm((8, 8, 64, M), BF16),
        vm((B, M), BF16),
        vm((B, M), BF16),
        vm((128, 128 * H), BF16),
        vm((B * H, D), F32),
        vm((HG, SK), F32),
        vm((HG, SK), F32),
        vm((HG, D), F32),
        vm((HG, HG, D), F32),
        vm((H, 8, D), F32),
        vm((B * H, M), BF16),
        vm((B * H, D), F32),
        vm((B * H, D), BF16),
        vm((B * H, M), BF16),
        vm((H, SK), F32),
        vm((H, SK), BF16),
        vm((H, D), F32),
        vm((H, M), F32),
        vm((H, 8, D), F32),
        pltpu.SemaphoreType.DMA((KS,)),
        pltpu.SemaphoreType.DMA((VS,)),
        pltpu.SemaphoreType.DMA((5,)),
        pltpu.SemaphoreType.DMA((6 + len(TAIL),)),
        pltpu.SemaphoreType.DMA((2,)),
    ]
    out = pl.pallas_call(
        _kernel,
        in_specs=[pl.BlockSpec(memory_space=pl.ANY)] * 11,
        out_specs=pl.BlockSpec(memory_space=pltpu.VMEM),
        out_shape=jax.ShapeDtypeStruct((B, 2 * M), A_x.dtype),
        scratch_shapes=scratch,
        compiler_params=pltpu.CompilerParams(
            vmem_limit_bytes=96 * 1024 * 1024,
            disable_bounds_checks=True,
            disable_semaphore_checks=True),
    )(*args)
    return out.reshape(B, 1, 2 * M)
```

```python
import jax
import jax.numpy as jnp
from jax import lax
import jax.experimental.pallas as pl
import jax.experimental.pallas.tpu as pltpu

F32 = jnp.float32
BF16 = jnp.bfloat16

B = 4
H = 32
SK = 4096
D = 128
M = 512
HG = 8
NG = B * H // HG
R = 512
NC = SK // R
NSTEP = NG * NC
LOOK = 2
VLAG = 6
KS = LOOK + 1
VS = LOOK + 1 + NC - VLAG
A0 = 16
SCALE = float(D) ** -0.5

NT = (((1,), (1,)), ((), ()))

PHA = 15
PHB = 17
SW = 4
SC = 8


def _pieces(width, t0, t1):
    per = width // 128
    out = []
    while t0 < t1:
        s, c = divmod(t0, per)
        if c == 0 and t1 - t0 >= per:
            n = (t1 - t0) // per
            out.append((pl.ds(s * 8, n * 8), pl.ds(0, width)))
            t0 += n * per
        else:
            e = min(t1, (s + 1) * per)
            out.append((pl.ds(s * 8, 8), pl.ds(c * 128, (e - t0) * 128)))
            t0 = e
    return out


TAIL = [(0, 4, 2), (4, 4, 2), (0, 4, 3), (4, 4, 3)]


def _kernel(
    xa_hbm, ckv_hbm, wqa_hbm, wuk_hbm, wuv_hbm, woa_hbm,
    xb_hbm, k_hbm, v_hbm, wqb_hbm, wob_hbm,
    out_ref,
    kbuf, vbuf, ckv, wqa, wuk, wuv, woa, wqb, wob, xa, xb,
    e_ref, qb_s, s_buf, p_buf, linv, acc, ob,
    ya, pacc, qa, qacc, qabs, sa, pa, linva, acca, oa,
    ksem, vsem, wsem, osem, xsem,
):
    cp = pltpu.make_async_copy

    def part(src, dst, lo, ph, sem):
        w = src.shape[-1]
        rects = _pieces(w, 0, ph) if lo else _pieces(w, ph, 32)
        return [cp(src.at[r], dst.at[r], sem) for r in rects]

    def kv_step(src, dst, sem, g, c):
        out = []
        wrap = (c + 1) // NC
        for u in range(2):
            for j in range(HG):
                k = j * 16 + 2 * c + u
                jn = j if u == 0 else (j + wrap) % HG
                kn = k + 1 if j < HG - 1 or u == 0 else (k + 1) % 128
                out.append(part(src.at[g * 128 + k], dst.at[j, u], False, PHB, sem))
                out.append(part(src.at[g * 128 + kn], dst.at[jn, u], True, PHB, sem))
        return out

    def k_step(u):
        slot = u % KS
        return kv_step(k_hbm, kbuf.at[slot], ksem.at[slot], u // NC, u % NC)

    def v_step(u):
        w = u - VLAG
        slot = w % VS
        return kv_step(v_hbm, vbuf.at[slot], vsem.at[slot], w // NC, u % NC)

    def ring_step(src, dst, sem, ph, ns):
        nb = src.shape[0]
        nv = 16 // ns

        def f(s):
            out = []
            for i in range(nv):
                for r in range(ns):
                    k = r * (nb // ns) + s * nv + i
                    kn = (k + 1) % nb if r == ns - 1 and i == nv - 1 else k + 1
                    out.append(part(src.at[k], dst.at[k], False, ph, sem))
                    out.append(part(src.at[kn], dst.at[kn], True, ph, sem))
            return out
        return f

    ckv_step = ring_step(ckv_hbm, ckv, wsem.at[0], PHA, SC)
    wqa_step = ring_step(wqa_hbm, wqa, wsem.at[1], PHA, SW)
    wuk_step = ring_step(wuk_hbm, wuk, wsem.at[2], PHA, SW)
    wuv_step = ring_step(wuv_hbm, wuv, wsem.at[3], PHA, SW)
    wqb_step = ring_step(wqb_hbm, wqb, wsem.at[4], PHB, SW)

    def wo_heads(src, dst, ph, semf, regions, hh):
        out = []
        if hh == 0:
            out += [part(src.at[r, 0], dst.at[r, 0], True, ph, semf(r, 0))
                    for r in regions]
        for k in (2 * hh, 2 * hh + 1):
            for r in regions:
                out.append(part(src.at[r, k], dst.at[r, k], False, ph, semf(r, hh)))
                if k < 7:
                    out.append(part(src.at[r, k + 1], dst.at[r, k + 1], True, ph,
                                    semf(r, (k + 1) // 2)))
        return out

    def woa_sem(r, hh):
        if hh < 2:
            return osem.at[4 + hh]
        i, = [i for i, (r0, nr, h) in enumerate(TAIL)
              if h == hh and r0 <= r < r0 + nr]
        return osem.at[6 + i]

    wob_step = lambda s: wo_heads(wob_hbm, wob, PHB, lambda r, hh: osem.at[hh],
                                  range(8), s)
    woa_step = lambda s: wo_heads(woa_hbm, woa, PHA, woa_sem, range(8), s)

    def woa_tail(lane):
        out = []
        for r0, nr, hh in TAIL:
            h = nr // 2
            out += wo_heads(woa_hbm, woa, PHA, woa_sem,
                            range(r0 + lane * h, r0 + (lane + 1) * h), hh)
        return out

    def issue(lane0, lane1):
        for i in range(max(len(lane0), len(lane1))):
            for lane, slots in enumerate((lane0, lane1)):
                if i < len(slots):
                    for c in slots[i]:
                        c.start(priority=lane)

    def wait_all(ref, sem):
        cp(ref, ref, sem).wait()

    def issue_pro(step0, n0, lo, hi):
        def body(s, carry):
            issue(step0(s), ckv_step(n0 + s))
            return carry
        lax.fori_loop(lo, hi, body, 0)

    variants = [
        (0, 3, lambda u: (k_step(u), ckv_step(13 + u))),
        (3, VLAG, lambda u: (k_step(u), wuv_step(u - 2))),
        (VLAG, NSTEP, lambda u: (k_step(u), v_step(u))),
    ] + [
        (NSTEP + s, NSTEP + s + 1,
         lambda u, s=s: (wob_step(s) if s < 4 else woa_step(s - 4),
                         v_step(NSTEP + s)))
        for s in range(VLAG)
    ] + [
        (NSTEP + VLAG, NSTEP + VLAG + 1, lambda u: (woa_tail(0), woa_tail(1))),
    ]

    def issue_static(u):
        for lo, hi, f in variants:
            if lo <= u < hi:
                issue(*f(u))

    def issue_dynamic(u, umin, umax):
        for lo, hi, f in sorted(variants, key=lambda v: v[0] - v[1]):
            if hi > umin and lo <= umax:
                pl.when(jnp.logical_and(u >= lo, u < hi))(
                    lambda f=f: issue(*f(u)))

    issue(wqb_step(0), ckv_step(0))
    xa_cp = cp(xa_hbm, xa, xsem.at[0])
    xb_cp = cp(xb_hbm, xb, xsem.at[1])
    xa_cp.start()
    xb_cp.start(priority=1)

    er = lax.broadcasted_iota(jnp.int32, (128, 1024), 0)
    ec = lax.broadcasted_iota(jnp.int32, (128, 1024), 1)
    for j in range(4):
        e_ref[:, j * 1024:(j + 1) * 1024] = jnp.where(
            (ec // H) + j * 32 == er, 1.0, 0.0).astype(BF16)
    ob[...] = jnp.zeros_like(ob)
    oa[...] = jnp.zeros_like(oa)

    issue_pro(wqb_step, 0, 1, 4)
    issue_pro(wqa_step, 4, 0, 2)

    xa_cp.wait()
    xb_cp.wait()
    xav = xa[...].astype(F32)
    for b in range(B):
        ya[b * H:(b + 1) * H, :] = jnp.broadcast_to(
            xav[b:b + 1, :], (H, M)).astype(BF16)
    xbv = xb[...]

    wait_all(wqb, wsem.at[4])
    qb = None
    for kc in range(4):
        w = wqb[16 * kc:16 * kc + 16].reshape(128, H * D)
        t = jnp.dot(xbv[:, kc * 128:(kc + 1) * 128], w,
                    preferred_element_type=F32)
        qb = t if qb is None else qb + t
    for h in range(H):
        qb_s[pl.ds(h, B, stride=H), :] = qb[:, h * D:(h + 1) * D]

    issue_pro(wqa_step, 4, 2, 4)
    issue_pro(wuk_step, 8, 0, 4)
    issue(wuv_step(0), ckv_step(12))
    for u in range(LOOK):
        issue_static(u)

    def hmask():
        r = lax.broadcasted_iota(jnp.int32, (128, 1024), 0)
        c = lax.broadcasted_iota(jnp.int32, (128, 1024), 1)
        return (r % H) == (c % H)

    def w_piece(w_ref, i):
        return w_ref[pl.ds(i * 4, 4)].reshape(1024, D)

    def e_piece(i):
        return e_ref[:, pl.ds(pl.multiple_of((i % 4) * 1024, 1024), 1024)]

    def accumulate(ref, t, first):
        @pl.when(first)
        def _():
            ref[...] = t

        @pl.when(jnp.logical_not(first))
        def _():
            ref[...] += t

    def proj_piece(w_ref, i):
        y = ya[:, pl.ds(pl.multiple_of((i // 4) * 128, 128), 128)]
        lx = jnp.dot(y, e_piece(i), preferred_element_type=F32)
        lx = jnp.where(hmask(), lx, 0.0).astype(BF16)
        accumulate(pacc, jnp.dot(lx, w_piece(w_ref, i),
                                 preferred_element_type=F32), i == 0)

    def qabs_piece(i):
        gx = lax.dot_general(qa[...], w_piece(wuk, i), NT,
                             preferred_element_type=F32)
        gx = jnp.where(hmask(), gx, 0.0)
        hi = gx.astype(BF16)
        lo = (gx - hi.astype(F32)).astype(BF16)
        t = lax.dot_general(jnp.concatenate([hi, lo], axis=0), e_piece(i), NT,
                            preferred_element_type=F32)
        accumulate(qacc, t, i % 4 == 0)

        @pl.when(i % 4 == 3)
        def _():
            col = pl.ds(pl.multiple_of((i // 4) * 128, 128), 128)
            for b in range(B):
                for z in range(2):
                    r = z * B * H + b * H
                    qabs[b, z * H:(z + 1) * H, col] = qacc[r:r + H, :].astype(BF16)

    def ckv_piece(b, c):
        return ckv[pl.ds((b * 4 + c) * 16, 16)].reshape(1024, M)

    def a_scores(b, c):
        t = lax.dot_general(qabs[b], ckv_piece(b, c), NT,
                            preferred_element_type=F32)
        sa[:, pl.ds(pl.multiple_of(c * 1024, 1024), 1024)] = t[0:H] + t[H:2 * H]

    def softmax(s_ref, p_ref, linv_ref):
        s = s_ref[...]
        m = jnp.max(s, axis=1, keepdims=True)
        p = jnp.exp((s - m) * SCALE)
        p_ref[...] = p.astype(p_ref.dtype)
        linv_ref[...] = jnp.broadcast_to(
            1.0 / jnp.sum(p, axis=1, keepdims=True), linv_ref.shape)

    def a_pv(b, c):
        p = pa[:, pl.ds(pl.multiple_of(c * 1024, 1024), 1024)]
        accumulate(acca, jnp.dot(p, ckv_piece(b, c),
                                 preferred_element_type=F32), c == 0)

    def a_piece(i):
        @pl.when(i == 0)
        def _():
            wait_all(wqa, wsem.at[1])
            wait_all(wuk, wsem.at[2])
            wait_all(wuv, wsem.at[3])
            wait_all(ckv, wsem.at[0])

        @pl.when(i < 16)
        def _():
            proj_piece(wqa, i)

            @pl.when(i == 15)
            def _():
                qa[...] = pacc[...].astype(BF16)

        @pl.when(jnp.logical_and(i >= 16, i < 32))
        def _():
            qabs_piece(i - 16)

        attn = jnp.logical_and(i >= 32, i < 64)
        b = (i - 32) // 8
        c = i % 8

        @pl.when(jnp.logical_and(attn, c < 4))
        def _():
            a_scores(b, c)

            @pl.when(c == 3)
            def _():
                softmax(sa, pa, linva)

        @pl.when(jnp.logical_and(attn, c >= 4))
        def _():
            a_pv(b, c - 4)

            @pl.when(c == 7)
            def _():
                li = jnp.concatenate([linva[...]] * 4, axis=1)
                ya[pl.ds(pl.multiple_of(b * H, H), H), :] = (
                    acca[...] * li).astype(BF16)

        @pl.when(i >= 64)
        def _():
            proj_piece(wuv, i - 64)

            @pl.when(i == 79)
            def _():
                for h in range(H):
                    oa[h, 0:B, :] = pacc[pl.ds(h, B, stride=H), :]

    def pv(w):
        slot = w % VS
        wait_all(vbuf.at[slot], vsem.at[slot])
        off = ((w + VLAG) % NC) * R
        if not isinstance(off, int):
            off = pl.multiple_of(off, R)
        p = p_buf[:, pl.ds(off, R)].astype(BF16)
        for j in range(HG):
            acc[j] += jnp.dot(p, vbuf[slot, j].reshape(R, D),
                              preferred_element_type=F32)

    def finish_group(g):
        for j in range(HG):
            o = acc[j] * linv[...]
            ob[(g % 4) * HG + j, pl.ds(g // 4, 1), :] = o[j:j + 1, :]

    def qk(t):
        slot = t % KS
        wait_all(kbuf.at[slot], ksem.at[slot])
        q = qb_s[pl.ds(pl.multiple_of((t // NC) * HG, HG), HG), :].astype(BF16)
        row = lax.broadcasted_iota(jnp.int32, (HG, R), 0)
        s = None
        for j in range(HG):
            r = lax.dot_general(q, kbuf[slot, j].reshape(R, D), NT,
                                preferred_element_type=F32)
            s = r if s is None else jnp.where(row == j, r, s)
        s_buf[:, pl.ds(pl.multiple_of((t % NC) * R, R), R)] = s

    def out_proj(o_ref, w_ref, heads, tot):
        for h in heads:
            t = jnp.dot(o_ref[h].astype(BF16),
                        w_ref[h // 4, 2 * (h % 4):2 * (h % 4) + 2].reshape(D, M),
                        preferred_element_type=F32)
            tot = t if tot is None else tot + t
        return tot

    def step(t, carry):
        issue_dynamic(t + LOOK, LOOK, NSTEP - 1 + LOOK)
        last = t % NC == NC - 1

        @pl.when(t >= NC)
        def _():
            pv(t - NC)

            @pl.when(last)
            def _():
                finish_group(t // NC - 1)

        qk(t)

        @pl.when(last)
        def _():
            softmax(s_buf, p_buf, linv)
            acc[...] = jnp.zeros_like(acc)

        @pl.when(jnp.logical_and(t >= A0, t < A0 + 80))
        def _():
            a_piece(t - A0)

        return carry

    lax.fori_loop(0, NSTEP, step, 0)

    late = range(H - HG, H)
    resa = resb = None
    w = NSTEP - NC
    for t in range(NSTEP, NSTEP + VLAG):
        issue_static(t + LOOK)
        while w <= t - VLAG:
            pv(w)
            w += 1
        s = t - NSTEP
        if s == VLAG - 1:
            finish_group(NG - 1)
            resb = out_proj(ob, wob, late, resb)
            out_ref[:, M:2 * M] = resb[0:B, :].astype(out_ref.dtype)
        if s < 4:
            wait_all(wob.at[:, pl.ds(2 * s, 2)], osem.at[s])
            resb = out_proj(ob, wob, [h for h in range(s, H, 4) if h not in late],
                            resb)
        else:
            wait_all(woa.at[:, pl.ds(2 * (s - 4), 2)], osem.at[s])
            resa = out_proj(oa, woa, range(s - 4, H, 4), resa)

    for i, (r0, nr, hh) in enumerate(TAIL):
        wait_all(woa.at[pl.ds(r0, nr), pl.ds(2 * hh, 2)], osem.at[6 + i])
        resa = out_proj(oa, woa, [4 * r + hh for r in range(r0, r0 + nr)], resa)
    out_ref[:, 0:M] = resa[0:B, :].astype(out_ref.dtype)


@jax.jit
def pallas_concat_heads__compressed_kv_cla__mha_block_cached__decode_kernel(
    A_x: jax.Array,
    A_c_kv: jax.Array,
    A_w_q: jax.Array,
    A_w_uk: jax.Array,
    A_w_uv: jax.Array,
    A_w_o: jax.Array,
    B_x: jax.Array,
    B_k_cache: jax.Array,
    B_v_cache: jax.Array,
    B_wq: jax.Array,
    B_wo: jax.Array,
):
    args = (
        A_x.reshape(B, M),
        A_c_kv.reshape(256, 64, M),
        A_w_q.reshape(64, 256, D),
        A_w_uk.reshape(64, 256, D),
        A_w_uv.reshape(64, 256, D),
        A_w_o.reshape(8, 8, 64, M),
        B_x.reshape(B, M),
        B_k_cache.reshape(2048, 256, D),
        B_v_cache.reshape(2048, 256, D),
        B_wq.reshape(64, 8, H * D),
        B_wo.reshape(8, 8, 64, M),
    )

    vm = pltpu.VMEM
    scratch = [
        vm((KS, HG, 2, 256, D), BF16),
        vm((VS, HG, 2, 256, D), BF16),
        vm((256, 64, M), BF16),
        vm((64, 256, D), BF16),
        vm((64, 256, D), BF16),
        vm((64, 256, D), BF16),
        vm((8, 8, 64, M), BF16),
        vm((64, 8, H * D), BF16),
        vm((8, 8, 64, M), BF16),
        vm((B, M), BF16),
        vm((B, M), BF16),
        vm((128, 128 * H), BF16),
        vm((B * H, D), F32),
        vm((HG, SK), F32),
        vm((HG, SK), F32),
        vm((HG, D), F32),
        vm((HG, HG, D), F32),
        vm((H, 8, D), F32),
        vm((B * H, M), BF16),
        vm((B * H, D), F32),
        vm((B * H, D), BF16),
        vm((2 * B * H, D), F32),
        vm((B, 2 * H, M), BF16),
        vm((H, SK), F32),
        vm((H, SK), BF16),
        vm((H, D), F32),
        vm((H, M), F32),
        vm((H, 8, D), F32),
        pltpu.SemaphoreType.DMA((KS,)),
        pltpu.SemaphoreType.DMA((VS,)),
        pltpu.SemaphoreType.DMA((5,)),
        pltpu.SemaphoreType.DMA((6 + len(TAIL),)),
        pltpu.SemaphoreType.DMA((2,)),
    ]
    out = pl.pallas_call(
        _kernel,
        in_specs=[pl.BlockSpec(memory_space=pl.ANY)] * 11,
        out_specs=pl.BlockSpec(memory_space=pltpu.VMEM),
        out_shape=jax.ShapeDtypeStruct((B, 2 * M), A_x.dtype),
        scratch_shapes=scratch,
        compiler_params=pltpu.CompilerParams(
            vmem_limit_bytes=96 * 1024 * 1024,
            disable_bounds_checks=True,
            disable_semaphore_checks=True),
    )(*args)
    return out.reshape(B, 1, 2 * M)
```
